```python
import os as _os
_os.environ.setdefault("JAX_PLATFORMS", "cpu")
import jax
import jax.numpy as jnp

def _softmax(x, axis=-1):
    return jax.nn.softmax(x, axis=axis)
def _gelu(x):
    return jax.nn.gelu(x, approximate=True)
def _silu(x):
    return jax.nn.silu(x)
def _sigmoid(x):
    return jax.nn.sigmoid(x)
def _layernorm(x, axis=-1, eps=1e-5):
    m = jnp.mean(x, axis=axis, keepdims=True)
    v = jnp.var(x, axis=axis, keepdims=True)
    return (x - m) / jnp.sqrt(v + eps)
def _scatter_add(tgt, idx, src, axis=0):
    return tgt.at[idx].add(src)
def _segment_sum(src, seg, n):
    return jax.ops.segment_sum(src, seg, n)
class _Rng:
    def __init__(self, key):
        self._k = key
    def _next(self):
        self._k, sub = jax.random.split(self._k)
        return sub
    def normal(self, shape):
        return jax.random.normal(self._next(), shape, dtype=jnp.bfloat16)
    def randint(self, lo, hi, shape):
        return jax.random.randint(self._next(), shape, lo, hi, dtype=jnp.int32)
    def uniform(self, shape, lo=0.0, hi=1.0):
        return jax.random.uniform(self._next(), shape, jnp.bfloat16, lo, hi)
    def permutation(self, n):
        return jax.random.permutation(self._next(), n)


kernel_name = 'parallel_sum__mha_block__dense_activation_mish__prompt'

def setup_inputs():
    _rng = _Rng(jax.random.key(int.from_bytes(__import__("os").urandom(4), "little")))
    _w = (lambda a: (lambda t: t.astype(jnp.bfloat16) if jnp.issubdtype(t.dtype, jnp.floating) else t)(jnp.asarray(a)))
    def _A_setup():
        B, S, D, H = 1, 2048, 512, 32
        return {
            "x": _w((lambda *s: _rng.normal(s) * 0.05)(B, S, D)),
            "wqkv": _w((lambda *s: _rng.normal(s) * 0.05)(D, 3 * D)),
            "wo": _w((lambda *s: _rng.normal(s) * 0.05)(D, D)),
        }
    _A_in = _A_setup()

    def _B_setup():
        B, S, D, F = 1, 2048, 512, 1792
        return {
            "x": _w((lambda *s: _rng.normal(s) * 0.05)(B, S, D)),
            "w1": _w((lambda *s: _rng.normal(s) * 1.6)(D, F) * (D ** -0.5)),
            "b1": _w((lambda *s: _rng.normal(s) * 0.05)(F)),
            "w2": _w((lambda *s: _rng.normal(s) * 0.05)(F, D) * (F ** -0.5)),
        }
    _B_in = _B_setup()

    return {
        "A_x": _A_in["x"],
        "A_wqkv": _A_in["wqkv"],
        "A_wo": _A_in["wo"],
        "B_x": _B_in["x"],
        "B_w1": _B_in["w1"],
        "B_b1": _B_in["b1"],
        "B_w2": _B_in["w2"],
    }

def reference(A_x, A_wqkv, A_wo, B_x, B_w1, B_b1, B_w2):
    def _A_ref(x, wqkv, wo):
        B, S, D = x.shape
        H = 32
        Dh = D // H
        qkv = (lambda x, *d: x.transpose(*d))((x @ wqkv).reshape(B, S, 3, H, Dh), 2, 0, 3, 1, 4)
        q, k, v = qkv[0], qkv[1], qkv[2]
        scores = jnp.einsum("bhqd,bhkd->bhqk", q, k) * (Dh ** -0.5)
        p = _softmax(scores, axis=-1)
        o = jnp.einsum("bhqk,bhkd->bhqd", p, v)
        return (lambda x, *d: x.transpose(*d))(o, 0, 2, 1, 3).reshape(B, S, D) @ wo

    def _B_ref(x, w1, b1, w2):
        h = jnp.einsum("bsd,df->bsf", x, w1) + b1
        sp = jnp.log1p(jnp.exp(-jnp.abs(h))) + jnp.where(h > 0, h, jnp.zeros_like(h))
        act = h * jnp.tanh(sp)
        return jnp.einsum("bsf,fd->bsd", act, w2)

    x = A_x
    xn = _layernorm(x, axis=-1)
    return x + _A_ref(xn, A_wqkv, A_wo) + _B_ref(xn, B_w1, B_b1, B_w2)
```

```python
import math
import jax
import jax.numpy as jnp
from jax import lax
import jax.experimental.pallas as pl
import jax.experimental.pallas.tpu as pltpu

H = 32
F32 = jnp.float32
BF16 = jnp.bfloat16
U32 = jnp.uint32
NT = (((1,), (1,)), ((), ()))


def pk(x):
  return pltpu.bitcast(x, U32)


def upk(x):
  return pltpu.bitcast(x, BF16)


def mish(hh):
  sp = jnp.log1p(jnp.exp(-jnp.abs(hh))) + jnp.maximum(hh, 0.0)
  return hh * jnp.tanh(sp)


def make(TQ=512, TK=128, UNROLL=1, RB=512, OB=256, flags=None, VPOS=4, LD=2, PIN=(0, 3), KP=8, KQ=0, XB=2, CB=1, JG=1,
         force_bad=False, P1U=True, P3U=False):
  NT_ = TK // 16
  NM = NT_ - 1
  NC = TQ // 128
  korder = list(range(NM))[:VPOS] + [NM] + list(range(NM))[VPOS:]

  def kernel(x_hbm, wqkv_hbm, wo_hbm, w1_hbm, b1_ref, w2_hbm, o_hbm,
             x_scr, wq_scr, wk_scr, wv_scr, wo_scr, w1_scr, w2_scr, o_scr,
             xn_scr, wqT, wvT, qT_scr, qf_scr, k_scr, kf_scr, vT_scr, oT_scr,
             kb_scr, p_scr, l_scr, acc_scr, one_scr, bad_scr, s_scr, z_smem, isem, osem):
    S, D = x_scr.shape
    Dh = D // H
    NQ = S // TQ
    NK = S // TK
    SP = NK * NQ
    NR = S // RB
    qscale = float(Dh ** -0.5 * math.log2(math.e))

    XR = RB // XB
    def x_copy(i):
      return pltpu.make_async_copy(x_hbm.at[pl.ds(i * XR, XR)], x_scr.at[pl.ds(i * XR, XR)], isem.at[i])
    nx = S // XR
    wk_cp = pltpu.make_async_copy(wqkv_hbm.at[:, pl.ds(D, D)], wk_scr, isem.at[nx])
    wq_cp = pltpu.make_async_copy(wqkv_hbm.at[:, pl.ds(0, D)], wq_scr, isem.at[nx + 1])
    wv_cp = pltpu.make_async_copy(wqkv_hbm.at[:, pl.ds(2 * D, D)], wv_scr, isem.at[nx + 2])
    late = [pltpu.make_async_copy(a, b, isem.at[nx + 3 + i])
            for i, (a, b) in enumerate(((w1_hbm, w1_scr), (w2_hbm, w2_scr), (wo_hbm, wo_scr)))]
    x_copy(0).start()
    wk_cp.start()
    for i in range(1, nx):
      x_copy(i).start()
    wq_cp.start()
    wv_cp.start()
    for cp in late:
      cp.start()

    with jax.named_scope('ph1a'):
      for i in range(nx):
        x_copy(i).wait()
        x = x_scr[i * XR:(i + 1) * XR, :].astype(F32)
        mu = jnp.mean(x, axis=-1, keepdims=True)
        xc = x - mu
        var = jnp.mean(xc * xc, axis=-1, keepdims=True)
        xn = (xc * lax.rsqrt(var + 1e-5)).astype(BF16)
        xn_scr[i * XR // 2:(i + 1) * XR // 2, :] = pk(xn)
        if i == 0:
          wk_cp.wait()
        k = jnp.dot(xn, wk_scr[...], preferred_element_type=F32).astype(BF16)
        for h in range(H):
          c, o = divmod(h * Dh, 128)
          kt = pk(k[:, c * 128:(c + 1) * 128])
          if o:
            kt = pltpu.roll(kt, 128 - o, 1)
          for t in range(XR // TK):
            j = i * (XR // TK) + t
            k_scr[h, j] = kt[t * TK // 2:t * TK // 2 + 8 * NM]
            kf_scr[h, j] = upk(kt[(t + 1) * TK // 2 - 8:(t + 1) * TK // 2]).astype(F32)
        if i == nx - 3:
          wq_cp.wait()
          wqT[...] = pk(wq_scr[...].astype(F32).T.astype(BF16))
        if i == nx - 2:
          wv_cp.wait()
          wvT[...] = pk(wv_scr[...].astype(F32).T.astype(BF16))

    def p1(r, c):
      xn = upk(xn_scr[pl.ds(r * (RB // 2) if P1U else pl.multiple_of(r * (RB // 2), RB // 2), RB // 2), :])
      qT = lax.dot_general(upk(wqT[...]), xn, NT, preferred_element_type=F32) * qscale
      xp = []
      for t in range(RB // TK):
        xp += [xn[t * TK + 16 * o:t * TK + 16 * o + 16] for o in korder[::-1]]
      vT = lax.dot_general(upk(wvT[...]), jnp.concatenate(xp, axis=0), NT, preferred_element_type=F32)
      for t in range(RB // TQ):
        qb = r * (RB // TQ) + t
        qT_scr[qb] = pk(qT[:, t * TQ:(t + 1) * TQ].astype(BF16)).reshape(H, Dh // 2, TQ)
        for cc in range(NC):
          qf_scr[:, qb * NC + cc] = qT[:, t * TQ + cc * 128:t * TQ + (cc + 1) * 128].reshape(H, Dh, 128)
      for t in range(RB // TK):
        vT_scr[:, r * (RB // TK) + t] = pk(vT[:, t * TK:(t + 1) * TK].astype(BF16)).reshape(H, Dh // 2, TK)
      return c
    with jax.named_scope('ph1b'):
      if P1U:
        for r in range(NR): p1(r, 0)
      else:
        lax.fori_loop(0, NR, p1, 0)

    for jj in range(JG):
      z_smem[jj] = 0
    one_scr[...] = jnp.ones(one_scr.shape, F32)
    bad_scr[...] = jnp.zeros(bad_scr.shape, F32)
    p_scr[...] = jnp.zeros(p_scr.shape, U32)
    l_scr[NQ - 1] = jnp.ones((8, TQ), F32)
    acc_scr[NQ - 1] = jnp.zeros((Dh, TQ), F32)

    def stage_keys(kf, slot):
      for d in range(Dh):
        kb_scr[slot, d] = jnp.broadcast_to(kf[:, d:d + 1], (16, 128))
    for jj in range(JG):
      stage_keys(kf_scr[0, jj], jj)

    def coords(r):
      jg, r2 = divmod(r, NQ * JG)
      qb, jj = divmod(r2, JG)
      return jg, qb, jj, jg * JG + jj

    def pv(h, r, p, acc, l):
      jg, qb, jj, j = coords(r)
      a = jnp.dot(upk(vT_scr[h, j]), p, preferred_element_type=F32)
      if jj > 0:
        a = acc + a
      elif j > 0:
        a = acc_scr[qb] + a
      if j == NK - 1:
        l = jnp.sum(l, axis=0, keepdims=True)
        ok = (l >= 2.0 ** -60) & (l <= 2.0 ** 60) & (jnp.abs(a) <= 2.0 ** 120)
        bad_scr[...] = jnp.where(ok, bad_scr[...], 1.0)
        oT_scr[qb, h] = pk((a / l).astype(BF16))
      elif jj == JG - 1:
        acc_scr[qb] = a
      return a

    def heads(h0, n):
      lh, sh = {}, {}
      always = one_scr[...] > 0

      def pin(x, slot, c):
        g2, t = divmod(slot, NT_)
        if slot < 0 or g2 not in sh: return x
        t = min(t, NM - 1)
        return jnp.where(always[:, :128], x, sh[g2][16 * t:16 * t + 8, c * 128:(c + 1) * 128])

      acc = pv_prev = None
      for g in range(n * SP):
        u, r = divmod(g, SP)
        jg, qb, jj, j = coords(r)
        par = (u * (NK // JG) + jg) % 2
        h = h0 + u
        hz = h + z_smem[jj] if JG > 1 else h
        qw = qT_scr[qb, hz]
        if LD and g - LD in lh:
          qw = jnp.where(always, qw, pk(lh[g - LD]))
        s = jnp.dot(upk(k_scr[h, j])[:, :Dh], upk(qw), preferred_element_type=F32)
        sh[g] = s
        sv = [[None] * NC for _ in range(2)]
        for c0 in range(0, NC, CB):
          for d in range(Dh):
            kd = kb_scr[par * JG + jj, d]
            for c in range(c0, c0 + CB):
              qd = qf_scr[hz, qb * NC + c, pl.ds(d, 8, stride=0), :]
              if d == 0:
                qd = pin(qd, NT_ * g + PIN[0] - PIN[1] * c0, c)
              for e in range(2):
                t_ = kd[8 * e:8 * e + 8] * qd
                sv[e][c] = t_ if d == 0 else sv[e][c] + t_
        sv = [jnp.concatenate(x, axis=1) for x in sv]
        jn, ph = divmod(r % (NQ * JG), NQ)
        if ph == KQ:
          j2 = (jg + 1) * JG + jn
          kf = kf_scr[h, j2] if j2 < NK else kf_scr[jnp.minimum(h + 1, H - 1), j2 - NK]
          kf = jnp.concatenate([pin(kf[8 * e:8 * e + 8], NT_ * g - KP, 0) for e in range(2)], axis=0)
          stage_keys(kf, (1 - par) * JG + jn)
        if g == 0:
          acc = pv(jnp.maximum(h0 - 1, 0), SP - 1, upk(p_scr[...]), acc_scr[NQ - 1], l_scr[NQ - 1])
        else:
          acc = pv(*pv_prev, acc, lh[g - 1])
        l = lh[g - 1] if jj > 0 else (l_scr[qb] if j > 0 else None)
        tiles = [None] * NT_
        for pos, t in enumerate(korder):
          s0, s1 = (s[16 * t:16 * t + 8], s[16 * t + 8:16 * t + 16]) if t < NM else sv
          p0, p1 = jnp.exp2(s0), jnp.exp2(s1)
          l = p0 if l is None else l + p0
          l = l + p1
          tiles[NT_ - 1 - pos] = jnp.concatenate([p0, p1], axis=0)
        lh[g] = l
        if jj == JG - 1 and j < NK - 1:
          l_scr[qb] = l
        pv_prev = (h, r, jnp.concatenate(tiles, axis=0).astype(BF16))
      p_scr[...] = pk(pv_prev[2])
      l_scr[NQ - 1] = l
      if JG > 1:
        acc_scr[NQ - 1] = acc

    def p2(i, c):
      heads(i * UNROLL, UNROLL)
      return c
    with jax.named_scope('ph2'):
      lax.fori_loop(0, H // UNROLL, p2, 0)
    pv(H - 1, SP - 1, upk(p_scr[...]), acc_scr[NQ - 1], l_scr[NQ - 1])

    @pl.when(jnp.max(bad_scr[...]) > (-1.0 if force_bad else 0.0))
    def _():
      def item(it, c):
        h, qb = it // NQ, it % NQ
        q = upk(qT_scr[qb, h])
        def scores(j, m):
          kt = jnp.concatenate([k_scr[h, j], pk(kf_scr[h, j].astype(BF16))], axis=0)
          kt = jnp.concatenate([kt[8 * o:8 * o + 8] for o in korder[::-1]], axis=0)
          s = jnp.dot(upk(kt)[:, :Dh], q, preferred_element_type=F32)
          s_scr[j] = s
          return jnp.maximum(m, jnp.max(s.reshape(TK // 8, 8, TQ), axis=0))
        m = lax.fori_loop(0, NK, scores, jnp.full((8, TQ), -jnp.inf, F32))
        m = jnp.max(m, axis=0, keepdims=True)
        def accum(j, carry):
          p = jnp.exp2(s_scr[j] - m)
          return (carry[0] + jnp.sum(p.reshape(TK // 8, 8, TQ), axis=0),
                  carry[1] + jnp.dot(upk(vT_scr[h, j]), p.astype(BF16), preferred_element_type=F32))
        l, a = lax.fori_loop(0, NK, accum, (jnp.zeros((8, TQ), F32), jnp.zeros((Dh, TQ), F32)))
        oT_scr[qb, h] = pk((a / jnp.sum(l, axis=0, keepdims=True)).astype(BF16))
        return c
      lax.fori_loop(0, H * NQ, item, 0)

    for cp in late:
      cp.wait()
    b1 = b1_ref[...].astype(F32).reshape(1, -1)

    def o_copy(i):
      return pltpu.make_async_copy(o_scr.at[pl.ds(i * OB, OB)], o_hbm.at[pl.ds(i * OB, OB)], osem.at[i])

    def p3(r, c):
      o = upk(oT_scr[r].reshape(D // 2, TQ)).astype(F32).T.astype(BF16)
      for t in range(TQ // OB):
        i = r * (TQ // OB) + t
        rows = pl.ds(i * OB if P3U else pl.multiple_of(i * OB, OB), OB)
        xn = upk(xn_scr[pl.ds(i * (OB // 2) if P3U else pl.multiple_of(i * (OB // 2), OB // 2), OB // 2), :])
        hh = jnp.dot(xn, w1_scr[...], preferred_element_type=F32) + b1
        y = jnp.dot(mish(hh).astype(BF16), w2_scr[...], preferred_element_type=F32)
        y = y + jnp.dot(o[t * OB:(t + 1) * OB], wo_scr[...], preferred_element_type=F32)
        o_scr[rows, :] = (x_scr[rows, :].astype(F32) + y).astype(o_scr.dtype)
        o_copy(i).start()
      return c
    with jax.named_scope('ph3'):
      if P3U:
        for r in range(NQ): p3(r, 0)
      else:
        lax.fori_loop(0, NQ, p3, 0)
    for i in range(S // OB):
      o_copy(i).wait()

  def fn(A_x, A_wqkv, A_wo, B_x, B_w1, B_b1, B_w2):
    B, S, D = A_x.shape
    Dh = D // H
    F = B_w1.shape[1]
    NQ, NK = S // TQ, S // TK
    any_ = pl.BlockSpec(memory_space=pl.ANY)
    out = pl.pallas_call(
        kernel,
        out_shape=jax.ShapeDtypeStruct((S, D), A_x.dtype),
        in_specs=[any_, any_, any_, any_, pl.BlockSpec(memory_space=pltpu.VMEM), any_],
        out_specs=any_,
        scratch_shapes=[
            pltpu.VMEM((S, D), BF16), pltpu.VMEM((D, D), BF16), pltpu.VMEM((D, D), BF16), pltpu.VMEM((D, D), BF16),
            pltpu.VMEM((D, D), BF16), pltpu.VMEM((D, F), BF16), pltpu.VMEM((F, D), BF16), pltpu.VMEM((S, D), BF16),
            pltpu.VMEM((S // 2, D), U32), pltpu.VMEM((D // 2, D), U32), pltpu.VMEM((D // 2, D), U32),
            pltpu.VMEM((NQ, H, Dh // 2, TQ), U32),
            pltpu.VMEM((H, S // 128, Dh, 128), F32),
            pltpu.VMEM((H, NK, 8 * NM, 128), U32),
            pltpu.VMEM((H, NK, 16, 128), F32),
            pltpu.VMEM((H, NK, Dh // 2, TK), U32),
            pltpu.VMEM((NQ, H, Dh // 2, TQ), U32),
            pltpu.VMEM((2 * JG, Dh, 16, 128), F32),
            pltpu.VMEM((TK // 2, TQ), U32),
            pltpu.VMEM((NQ, 8, TQ), F32), pltpu.VMEM((NQ, Dh, TQ), F32),
            pltpu.VMEM((8, TQ), F32), pltpu.VMEM((Dh, TQ), F32),
            pltpu.VMEM((NK, TK, TQ), F32),
            pltpu.SMEM((JG,), jnp.int32),
            pltpu.SemaphoreType.DMA((S // (RB // XB) + 6,)), pltpu.SemaphoreType.DMA((S // OB,)),
        ],
        compiler_params=pltpu.CompilerParams(vmem_limit_bytes=100 * 2**20, flags=flags),
    )(A_x.reshape(S, D), A_wqkv, A_wo, B_w1, B_b1, B_w2)
    return out.reshape(B, S, D)
  return fn


@jax.jit
def pallas_parallel_sum__mha_block__dense_activation_mish__prompt_kernel(A_x, A_wqkv, A_wo, B_x, B_w1, B_b1, B_w2):
  return make(JG=1,UNROLL=2)(A_x, A_wqkv, A_wo, B_x, B_w1, B_b1, B_w2)
```

```python
import math

import jax
import jax.numpy as jnp
from jax import lax
import jax.experimental.pallas as pl
import jax.experimental.pallas.tpu as pltpu

F32 = jnp.float32
BF16 = jnp.bfloat16
U32 = jnp.uint32

HEADS = 32
LANES = 128
TQ = 512
TK = 128
RB = 256
NC = TQ // LANES
NG = TK // 16
NM = NG - 1
X_CHUNKS = (256, 256, 512, 1024)

VPU_POS = 3
EXTRA_TILES = (4, 9, 15)
CHAIN_SLOT = (1, 3)
EXTRA_SLOT, EXTRA_DUE, EXTRA_SPAN, EXTRA_STAGE = -3, 3, (0, -1), 1
KEY_STAGE, KEY_LEAD, QUERY_LEAD = (0, 6, 11, 16, 16), 4, 16
FINISH_STEPS, FINISH_DUE = (42, 46, 50, 54), 3
PROJ_ORDER = "T n4 q1 s2 v0 n5 k4 s3 k5 W7 v1 s4 n6 q2 s5 n7 k6 v2 s6 k7 q3 s7 v3"

GROUP_ORDER = list(range(VPU_POS)) + [NM] + list(range(VPU_POS, NM))
P_ROWS = [16 * g + 8 * e for g in GROUP_ORDER[::-1] for e in (1, 0)]


def _pack(x):
  return pltpu.bitcast(x, U32)


def _unpack(x):
  return pltpu.bitcast(x, BF16)


def _dot(a, b):
  return jnp.dot(a, b, preferred_element_type=F32)


def _dot_nt(a, b):
  return lax.dot_general(a, b, (((1,), (1,)), ((), ())), preferred_element_type=F32)


def _after(true, x, dep):
  if dep.dtype != x.dtype:
    dep = pltpu.bitcast(dep, x.dtype)
  return jnp.where(true[:, :x.shape[1]], x, dep)


def _mish(h):
  w = jnp.exp(jnp.minimum(h, 20.0))
  n = w * (w + 2.0)
  d = n + 2.0
  r = pl.reciprocal(d, approx=True)
  return (h * (n * r)) * (2.0 - d * r)


def _strassen_lhs(a11, a12, a21, a22):
  return [a11 + a22, a21 + a22, a11, a22, a11 + a12, a21 - a11, a12 - a22]


def _strassen_rhs(b11, b12, b21, b22):
  return [b11 + b22, b11, b12 - b22, b21 - b11, b22, b11 + b12, b21 + b22]


STRASSEN_ORDER = (0, 3, 4, 6, 2, 1, 5)


def _strassen_blocks(prod):
  m = {i: prod(i) for i in STRASSEN_ORDER}
  return (m[0] + m[3] - m[4] + m[6], m[4] + m[2], m[3] + m[1], m[0] + m[2] - m[1] + m[5])


def _kernel(x_hbm, wqkv_hbm, wo_hbm, w1_hbm, b1_hbm, w2_hbm, out_hbm,
            x_ref, wq_ref, wk_ref, wv_ref, wo_ref, w1_ref, w2_ref, out_ref,
            wqT_ref, wvT_ref, xn_ref, xs_ref, w1s_ref, w2s_ref, wos_ref,
            qT_ref, k_ref, kv_ref, kx_ref, vT_ref, oT_ref,
            qa_ref, qb_ref, kb_ref, sx_ref, p_ref, l_ref, acc_ref, one_ref, bad_ref,
            s_ref, m_ref, b1_ref, in_sem, out_sem):
  S, D = x_ref.shape
  Dh = D // HEADS
  NQ, NK = S // TQ, S // TK
  hd, hf = D // 2, w1_ref.shape[1] // 2
  q_scale = Dh ** -0.5 * math.log2(math.e)

  copies = []

  def in_copy(src, dst):
    copies.append(pltpu.make_async_copy(src, dst, in_sem.at[len(copies)]))
    return copies[-1]

  def x_copy(i):
    rows = pl.ds(sum(X_CHUNKS[:i]), X_CHUNKS[i])
    return in_copy(x_hbm.at[rows], x_ref.at[rows])

  def start_copies(n):
    for _ in range(n):
      unstarted.pop(0).start()

  x0_cp = x_copy(0)
  wk_cp = [in_copy(wqkv_hbm.at[:, pl.ds(D + i * hd, hd)], wk_ref.at[:, pl.ds(i * hd, hd)]) for i in range(2)]
  x1_cp, x2_cp = x_copy(1), x_copy(2)
  wq_cp = in_copy(wqkv_hbm.at[:, pl.ds(0, D)], wq_ref)
  wv_cp = in_copy(wqkv_hbm.at[:, pl.ds(2 * D, D)], wv_ref)
  x3_cp = x_copy(3)
  late_cp = [in_copy(wo_hbm, wo_ref), in_copy(w1_hbm, w1_ref), in_copy(w2_hbm, w2_ref), in_copy(b1_hbm, b1_ref)]
  unstarted = list(copies)
  start_copies(4)
  one_ref[...] = jnp.ones(one_ref.shape, F32)

  def norm(r0):
    x = x_ref[r0:r0 + RB, :].astype(F32)
    xc = x - jnp.mean(x, axis=-1, keepdims=True)
    xn = xc * lax.rsqrt(jnp.mean(xc * xc, axis=-1, keepdims=True) + 1e-5)
    xn_ref[r0:r0 + RB, :] = xn.astype(BF16)
    for t in range(0, RB // 2, 16):
      top, bot = xn[t:t + 16], xn[RB // 2 + t:RB // 2 + t + 16]
      for i, op in enumerate(_strassen_lhs(top[:, :hd], top[:, hd:], bot[:, :hd], bot[:, hd:])):
        xs_ref[i, r0 // 2 + t:r0 // 2 + t + 16, :] = op.astype(BF16)

  def weight_jobs(w_ref, dst_ref):
    r, c = dst_ref.shape[1:]
    for t in range(0, r, 8):
      for u in range(0, c, 2 * LANES):
        def job(t=t, u=u, n=min(2 * LANES, c - u)):
          ops = _strassen_rhs(*[w_ref[i * r + t:i * r + t + 8, j * c + u:j * c + u + n].astype(F32)
                                for i in range(2) for j in range(2)])
          for i, op in enumerate(ops):
            dst_ref[i, t:t + 8, u:u + n] = op.astype(BF16)
          return (ops[0] + ops[6])[:, :LANES]
        yield job

  jobs, jobs_per_dot = [], 0

  def with_jobs(x):
    n = min(jobs_per_dot, len(jobs))
    if not n:
      return _unpack(x)
    true = one_ref[:, :LANES] > 0
    parts = [x[t:t + 8, :LANES] for t in range(0, x.shape[0], 8)]
    for i in range(n):
      t = i * len(parts) // n
      parts[t] = _after(true, parts[t], jobs.pop(0)())
    return _unpack(jnp.concatenate([jnp.concatenate(parts, axis=0), x[:, LANES:]], axis=1))

  def project_k(r0):
    xn = xn_ref[r0:r0 + RB, :]
    return _dot(with_jobs(_pack(xn)) if jobs else xn, wk_ref[...]).astype(BF16)

  def store_k(r0, k):
    for h in range(HEADS):
      c, off = divmod(h * Dh, LANES)
      kt = _pack(k[:, c * LANES:(c + 1) * LANES])
      if off:
        kt = pltpu.roll(kt, LANES - off, 1)
      for t in range(RB // TK):
        j, tile = r0 // TK + t, kt[t * TK // 2:(t + 1) * TK // 2]
        k_ref[h, j] = tile[:8 * NM]
        kv_ref[h, j] = _unpack(tile[8 * NM:]).astype(F32)
        if j in EXTRA_TILES:
          kx_ref[h, EXTRA_TILES.index(j)] = _unpack(tile[8 * (NM - 1):8 * NM]).astype(F32)

  def project_q(qb):
    qT = _dot_nt(with_jobs(wqT_ref[...]), xn_ref[qb * TQ:(qb + 1) * TQ, :]) * q_scale
    qT_ref[qb] = qT.reshape(HEADS, Dh, TQ)

  def project_v(qb):
    xn = jnp.concatenate([xn_ref[t + o:t + o + 8, :]
                          for t in range(qb * TQ, (qb + 1) * TQ, TK) for o in P_ROWS], axis=0)
    vT = _dot_nt(with_jobs(wvT_ref[...]), xn)
    for t in range(TQ // TK):
      vT_ref[:, qb * (TQ // TK) + t] = vT[:, t * TK:(t + 1) * TK].reshape(HEADS, Dh, TK)

  def transpose(w_ref, dst_ref):
    for c in range(0, D, LANES):
      dst_ref[:, c:c + LANES] = _pack(w_ref[c:c + LANES, :].astype(F32).T.astype(BF16))

  x0_cp.wait()
  start_copies(1)
  norm(0)
  wk_cp[0].wait()
  k_left = _dot(xn_ref[0:RB, :], wk_ref[:, :hd]).astype(BF16)
  wk_cp[1].wait()
  x1_cp.wait()
  start_copies(1)
  ks = {0: jnp.concatenate([k_left, _dot(xn_ref[0:RB, :], wk_ref[:, hd:]).astype(BF16)], axis=1)}
  norm(RB)
  x2_cp.wait()
  start_copies(2)
  store_k(0, ks.pop(0))
  ks[1] = project_k(RB)
  norm(2 * RB)
  ks[2] = project_k(2 * RB)
  norm(3 * RB)
  wq_cp.wait()
  start_copies(2)
  transpose(wq_ref, wqT_ref)
  ks[3] = project_k(3 * RB)
  store_k(RB, ks.pop(1))
  project_q(0)
  wv_cp.wait()
  x3_cp.wait()
  start_copies(2)
  for op in PROJ_ORDER.split():
    kind, n = op[0], int(op[1:] or 0)
    if kind == "T":
      transpose(wv_ref, wvT_ref)
    elif kind == "n":
      norm(n * RB)
    elif kind == "k":
      ks[n] = project_k(n * RB)
    elif kind == "s":
      store_k(n * RB, ks.pop(n))
    elif kind == "q":
      project_q(n)
    elif kind == "v":
      project_v(n)
    else:
      for cp in late_cp:
        cp.wait()
      for w_ref, dst_ref in ((wo_ref, wos_ref), (w1_ref, w1s_ref), (w2_ref, w2s_ref)):
        jobs.extend(weight_jobs(w_ref, dst_ref))
      jobs_per_dot = -(-len(jobs) // n)
  assert not (jobs or ks or unstarted)

  steps = NK * NQ
  bad_ref[...] = jnp.zeros(bad_ref.shape, F32)
  p_ref[...] = jnp.zeros(p_ref.shape, F32)
  l_ref[...] = jnp.ones(l_ref.shape, F32)
  acc_ref[...] = jnp.zeros(acc_ref.shape, F32)

  def stage_keys(k16, slot, dims):
    for d in dims:
      kb_ref[slot, d] = jnp.broadcast_to(k16[:, d:d + 1], (16, LANES))

  def stage_queries(tab_ref, q8, col, d0, rows):
    for d in rows:
      tab_ref[col, d0 + d] = jnp.broadcast_to(q8[d:d + 1], (8, LANES))

  def vpu_scores(slot, tab_ref, col, hold):
    out = [None, None]
    for d in range(Dh):
      k, q = kb_ref[slot, d], tab_ref[col, d]
      if d == 0:
        q = hold(q)
      for e in range(2):
        term = k[8 * e:8 * e + 8] * q
        out[e] = term if d == 0 else out[e] + term
    return out

  def extra_scores(slot, tab_ref, col, hold):
    out = vpu_scores(slot, tab_ref, col, hold)
    for e in range(2):
      sx_ref[col // NC, 8 * e:8 * e + 8, (col % NC) * LANES:(col % NC + 1) * LANES] = out[e]
    return out

  def add_pv(u, h, r, p):
    j, qb = divmod(r, NQ)
    a = _dot(vT_ref[h, j], p)
    acc_ref[u, qb] = acc_ref[u, qb] + a if j > 0 else a

  def finish(u, h, qb, l):
    a = acc_ref[u, qb]
    l = jnp.broadcast_to(jnp.sum(l, axis=0, keepdims=True), (8, TQ))
    ok = (l >= 2.0 ** -60) & (l <= 2.0 ** 60) & (jnp.abs(a[:8]) + jnp.abs(a[8:]) <= 2.0 ** 120)
    bad = jnp.where(ok, bad_ref[...], 1.0)
    bad_ref[...] = bad
    inv = 1.0 / l
    lo, hi = a[:8] * inv, a[8:] * inv
    oT_ref[qb, h] = jnp.concatenate([lo, hi], axis=0)
    return lo + hi + bad

  stage_keys(kv_ref[0, 0], 0, range(Dh))
  stage_keys(kx_ref[0, 0], 2, range(Dh))
  for col in range(NQ * NC):
    for d0 in range(0, Dh, 8):
      q8 = qT_ref[col // NC, 0, d0:d0 + 8, (col % NC) * LANES:(col % NC + 1) * LANES]
      stage_queries(qa_ref, q8, col, d0, range(8))

  def head_pair(i, carry):
    true = one_ref[...] > 0
    scores, finished, extras = {}, {}, {}

    def from_slot(slot, c=0):
      if slot < 0:
        return lambda x: x
      s = scores[slot // NG]
      t = min(slot % NG, s.shape[0] // 16 - 1)
      return lambda x: _after(true, x, s[16 * t:16 * t + 8, c * LANES:(c + 1) * LANES])

    def hold_keys(k16, g):
      return jnp.concatenate([from_slot(NG * g - KEY_LEAD)(k16[e:e + 8]) for e in (0, 8)], axis=0)

    pending = [(1, jnp.maximum(2 * i - 1, 0), steps - 1, p_ref[...])]
    for g in range(2 * steps):
      u, r = divmod(g, steps)
      j, qb = divmod(r, NQ)
      h = 2 * i + u
      h_next = jnp.minimum(h + 1, HEADS - 1)
      tab_ref, tab_next = (qa_ref, qb_ref) if u == 0 else (qb_ref, qa_ref)

      q = qT_ref[qb, h]
      q_lo, q_hi = q[:8], q[8:]
      if g - FINISH_DUE in finished:
        q_lo = _after(true, q_lo, finished[g - FINISH_DUE])
      if g - EXTRA_DUE in extras:
        dep = jnp.concatenate(extras[g - EXTRA_DUE], axis=1)
        n = dep.shape[1]
        q_hi = jnp.concatenate([_after(true, q_hi[:, :n], dep)] + ([q_hi[:, n:]] if n < TQ else []), axis=1)
      q = jnp.concatenate([q_lo, q_hi], axis=0)

      n_mxu = NM - 1 if j in EXTRA_TILES else NM
      mxu_scores = lambda a, b: _dot(_unpack(k_ref[h, j, 8 * a:8 * b])[:, :Dh], q)
      if g > 0:
        s = mxu_scores(0, NG - n_mxu)
        add_pv(*pending.pop(0))
        s = jnp.concatenate([s, mxu_scores(NG - n_mxu, n_mxu)], axis=0)
      else:
        s = mxu_scores(0, n_mxu)
      scores[g] = s

      sv = [vpu_scores(j % 2, tab_ref, qb * NC + c, from_slot(NG * g + CHAIN_SLOT[0] - CHAIN_SLOT[1] * c, c))
            for c in range(NC)]
      sv = [jnp.concatenate([x[e] for x in sv], axis=1) for e in range(2)]
      seg = sum(j > t for t in EXTRA_TILES)
      j0 = EXTRA_TILES[seg - 1] + 1 if seg else 0
      pos, span = r - j0 * NQ, (EXTRA_TILES[seg] - j0) * NQ + EXTRA_SPAN[1] - EXTRA_SPAN[0]
      par = (u * len(EXTRA_TILES) + seg) % 2
      for col in range(NQ * NC):
        if EXTRA_SPAN[0] + col * span // (NQ * NC) == pos:
          hold = from_slot(NG * g + EXTRA_SLOT - 2 * len(extras.get(g, [])))
          extras.setdefault(g, []).extend(extra_scores(2 + par, tab_ref, col, hold))

      if qb == NQ - 1 and 0 <= pos // NQ - EXTRA_STAGE < 4:
        k16 = kx_ref[h, seg + 1] if seg + 1 < len(EXTRA_TILES) else kx_ref[h_next, 0]
        d0 = 4 * (pos // NQ - EXTRA_STAGE)
        stage_keys(hold_keys(k16, g), 3 - par, range(d0, d0 + 4))
      if KEY_STAGE[qb] < KEY_STAGE[qb + 1]:
        k16 = kv_ref[h, j + 1] if j + 1 < NK else kv_ref[h_next, 0]
        stage_keys(hold_keys(k16, g), (j + 1) % 2, range(KEY_STAGE[qb], KEY_STAGE[qb + 1]))
      d0 = 8 * (qb // 2)
      q8 = qT_ref[j // NC, h_next, d0:d0 + 8, (j % NC) * LANES:(j % NC + 1) * LANES]
      stage_queries(tab_next, from_slot(NG * g - QUERY_LEAD, 1)(q8),
                    j + i // HEADS,
                    d0, range(4 * (qb % 2), 4 * (qb % 2) + 4))

      if g == 2 * steps - 1:
        add_pv(*pending.pop(0))
      if r in FINISH_STEPS:
        fq = FINISH_STEPS.index(r)
        l = jnp.concatenate([from_slot(NG * g - NG, c)(l_ref[1 - u, fq, :, c * LANES:(c + 1) * LANES])
                             for c in range(NC)], axis=1)
        finished[g] = finish(1 - u, jnp.maximum(h - 1, 0), fq, l)

      l = l_ref[u, qb] if j > 0 else None
      p = []
      for t in GROUP_ORDER:
        if t < n_mxu:
          halves = s[16 * t:16 * t + 8], s[16 * t + 8:16 * t + 16]
        else:
          halves = sv if t == NM else (sx_ref[qb, 0:8], sx_ref[qb, 8:16])
        for half in halves:
          p.append(jnp.exp2(half))
          l = p[-1] if l is None else l + p[-1]
      l_ref[u, qb] = l
      pending.append((u, h, r, jnp.concatenate(p[::-1], axis=0)))
    p_ref[...] = pending.pop()[3]
    return carry

  lax.fori_loop(0, HEADS // 2, head_pair, 0)
  add_pv(1, HEADS - 1, steps - 1, p_ref[...])
  for qb in range(NQ):
    finish(1, HEADS - 1, qb, l_ref[1, qb])

  @pl.when(jnp.max(bad_ref[...]) > 0)
  def _():
    def redo(it, carry):
      h, qb = it // NQ, it % NQ
      q = qT_ref[qb, h]

      def score_tile(j, m):
        k = jnp.concatenate([k_ref[h, j], _pack(kv_ref[h, j].astype(BF16))], axis=0)
        s = _dot(_unpack(k)[:, :Dh], q)
        s = jnp.concatenate([s[o:o + 8] for o in P_ROWS], axis=0)
        s_ref[j] = s
        return jnp.maximum(m, jnp.max(s.reshape(TK // 8, 8, TQ), axis=0))

      m = lax.fori_loop(0, NK, score_tile, jnp.full((8, TQ), -jnp.inf, F32))
      m = jnp.max(m, axis=0, keepdims=True)

      def pv_tile(j, sums):
        p = jnp.exp2(s_ref[j] - m)
        return sums[0] + jnp.sum(p.reshape(TK // 8, 8, TQ), axis=0), sums[1] + _dot(vT_ref[h, j], p)

      l, a = lax.fori_loop(0, NK, pv_tile, (jnp.zeros((8, TQ), F32), jnp.zeros((Dh, TQ), F32)))
      oT_ref[qb, h] = a / jnp.sum(l, axis=0, keepdims=True)
      return carry

    lax.fori_loop(0, HEADS * NQ, redo, 0)

  b1 = b1_ref[...].astype(F32).reshape(1, -1)

  def out_copy(i):
    rows = pl.ds(i * RB, RB)
    return pltpu.make_async_copy(out_ref.at[rows], out_hbm.at[rows], out_sem.at[i])

  def out_block(r, carry):
    m = TQ // 2
    xs = [xs_ref[i, pl.ds(pl.multiple_of(r * m, m), m), :] for i in range(7)]

    def hidden(c0, between):
      def prod(i):
        y = _dot(xs[i], w1s_ref[i, :, c0:c0 + LANES])
        between(i)
        return y
      act = [_mish(h + b1[:, (n % 2) * hf + c0:(n % 2) * hf + c0 + LANES])
             for n, h in enumerate(_strassen_blocks(prod))]
      ops = [op.astype(BF16) for op in _strassen_lhs(*act)]
      return lambda i, rows=slice(None): _dot(ops[i][rows], w2s_ref[i, c0:c0 + LANES, :])

    share = hidden(0, lambda i: None)
    o = oT_ref[r].reshape(D, TQ).T
    top, bot = [jnp.concatenate([o[t + e * RB // 2:t + (e + 1) * RB // 2] for t in range(0, TQ, RB)], axis=0)
                for e in range(2)]
    ops = _strassen_lhs(top[:, :hd], top[:, hd:], bot[:, :hd], bot[:, hd:])
    for i in STRASSEN_ORDER:
      m_ref[i] = _dot(ops[i].astype(BF16), wos_ref[i])
    for c0 in range(LANES, hf, LANES):
      def add_share(i, share=share):
        m_ref[i] += share(i)
      share = hidden(c0, add_share)
    for t in range(TQ // RB):
      sub = slice(t * RB // 2, (t + 1) * RB // 2)
      y = _strassen_blocks(lambda i: m_ref[i, sub] + share(i, sub))
      for e in range(2):
        rows = pl.ds(pl.multiple_of(r * TQ + t * RB + e * (RB // 2), RB // 2), RB // 2)
        res = x_ref[rows, :].astype(F32) + jnp.concatenate(y[2 * e:2 * e + 2], axis=1)
        out_ref[rows, :] = res.astype(out_ref.dtype)
      out_copy(r * (TQ // RB) + t).start()
    return carry

  lax.fori_loop(0, NQ, out_block, 0)
  for i in range(S // RB):
    out_copy(i).wait()


@jax.jit
def pallas_parallel_sum__mha_block__dense_activation_mish__prompt_kernel(
    A_x: jax.Array,
    A_wqkv: jax.Array,
    A_wo: jax.Array,
    B_x: jax.Array,
    B_w1: jax.Array,
    B_b1: jax.Array,
    B_w2: jax.Array,
):
  del B_x
  B, S, D = A_x.shape
  F = B_w1.shape[1]
  assert (B, S, D) == (1, sum(X_CHUNKS), 16 * HEADS) and F % (2 * LANES) == 0
  Dh, NQ, NK = D // HEADS, S // TQ, S // TK
  vmem = pltpu.VMEM
  hbm = pl.BlockSpec(memory_space=pl.ANY)
  out = pl.pallas_call(
      _kernel,
      out_shape=jax.ShapeDtypeStruct((S, D), A_x.dtype),
      in_specs=[hbm] * 6,
      out_specs=hbm,
      scratch_shapes=[
          vmem((S, D), A_x.dtype),
          *[vmem((D, D), A_wqkv.dtype)] * 3, vmem((D, D), A_wo.dtype),
          vmem((D, F), B_w1.dtype), vmem((F, D), B_w2.dtype), vmem((S, D), A_x.dtype),
          *[vmem((D // 2, D), U32)] * 2,
          vmem((S, D), BF16), vmem((7, S // 2, D // 2), BF16),
          vmem((7, D // 2, F // 2), BF16), vmem((7, F // 2, D // 2), BF16), vmem((7, D // 2, D // 2), BF16),
          vmem((NQ, HEADS, Dh, TQ), F32),
          vmem((HEADS, NK, 8 * NM, LANES), U32),
          vmem((HEADS, NK, 16, LANES), F32), vmem((HEADS, 4, 16, LANES), F32),
          vmem((HEADS, NK, Dh, TK), F32), vmem((NQ, HEADS, Dh, TQ), F32),
          *[vmem((S // LANES, Dh, 8, LANES), F32)] * 2, vmem((4, Dh, 16, LANES), F32),
          vmem((NQ, 16, TQ), F32), vmem((TK, TQ), F32),
          vmem((2, NQ, 8, TQ), F32), vmem((2, NQ, Dh, TQ), F32),
          vmem((8, TQ), F32), vmem((8, TQ), F32),
          vmem((NK, TK, TQ), F32), vmem((7, TQ // 2, D // 2), F32),
          vmem((F,), B_b1.dtype),
          pltpu.SemaphoreType.DMA((12,)), pltpu.SemaphoreType.DMA((S // RB,)),
      ],
      compiler_params=pltpu.CompilerParams(vmem_limit_bytes=100 * 2**20),
  )(A_x.reshape(S, D), A_wqkv, A_wo, B_w1, B_b1, B_w2)
  return out.reshape(B, S, D)
```

```python
import math

import jax
import jax.numpy as jnp
from jax import lax
import jax.experimental.pallas as pl
import jax.experimental.pallas.tpu as pltpu

F32 = jnp.float32
BF16 = jnp.bfloat16
U32 = jnp.uint32

HEADS = 32
LANES = 128
TQ = 512
TK = 128
RB = 256
NC = TQ // LANES
NG = TK // 16
NM = NG - 1
JOB_ROWS = 16
X_CHUNKS = (256, 256, 512, 1024)

PROJ_ORDER = "T q1 s2 n4 s3 v0 n5 k4 k5 W7 v1 s4 n6 s5 q2 n7 k6 v2 s6 k7 q3 s7 v3"

VPU_POS = 3
CHAIN_SLOT = (1, -3, -5, -9)
EXTRA_TILES = (4, 9, 15)
EXTRA_SLOT, EXTRA_DUE = -5, 3
KEY_STAGE = (0, 6, 13, 16, 16)
KEY_LEAD, QUERY_LEAD = 4, 7
FINISH_STEPS, FINISH_DUE = (42, 46, 49, 54), 3

GROUP_ORDER = list(range(VPU_POS)) + [NM] + list(range(VPU_POS, NM))
P_ROWS = [16 * g + 8 * e for g in GROUP_ORDER[::-1] for e in (1, 0)]


def _pack(x):
  return pltpu.bitcast(x, U32)


def _unpack(x):
  return pltpu.bitcast(x, BF16)


def _dot(a, b):
  return jnp.dot(a, b, preferred_element_type=F32)


def _dot_nt(a, b):
  return lax.dot_general(a, b, (((1,), (1,)), ((), ())), preferred_element_type=F32)


def _after(true, x, dep):
  if dep.dtype != x.dtype:
    dep = pltpu.bitcast(dep, x.dtype)
  return lax.select(true if true.shape == x.shape else true[:, :x.shape[1]], x, dep)


def _mish(h):
  w = jnp.exp(jnp.minimum(h, 20.0))
  n = w * (w + 2.0)
  d = n + 2.0
  r = pl.reciprocal(d, approx=True)
  return (h * (n * r)) * (2.0 - d * r)


def _strassen_lhs(a11, a12, a21, a22):
  return [a11 + a22, a21 + a22, a11, a22, a11 + a12, a21 - a11, a12 - a22]


def _strassen_rhs(b11, b12, b21, b22):
  return [b11 + b22, b11, b12 - b22, b21 - b11, b22, b11 + b12, b21 + b22]


STRASSEN_ORDER = (0, 3, 4, 6, 2, 1, 5)


def _strassen_blocks(prod):
  m = {i: prod(i) for i in STRASSEN_ORDER}
  return (m[0] + m[3] - m[4] + m[6], m[4] + m[2], m[3] + m[1], m[0] + m[2] - m[1] + m[5])


def _kernel(x_hbm, wqkv_hbm, wo_hbm, w1_hbm, b1_hbm, w2_hbm, out_hbm,
            x_ref, wq_ref, wk_ref, wv_ref, wo_ref, w1_ref, w2_ref, out_ref,
            wqT_ref, wvT_ref, xn_ref, xs_ref, w1s_ref, w2s_ref, wos_ref,
            qT_ref, k_ref, kv_ref, kx_ref, vT_ref, oT_ref,
            qa_ref, qb_ref, kb_ref, sx_ref, p_ref, l_ref, acc_ref, one_ref, bad_ref,
            s_ref, m_ref, b1_ref, in_sem, out_sem):
  S, D = x_ref.shape
  Dh = D // HEADS
  NQ, NK = S // TQ, S // TK
  hd, hf = D // 2, w1_ref.shape[1] // 2
  q_scale = Dh ** -0.5 * math.log2(math.e)

  copies = []

  def in_copy(src, dst):
    copies.append(pltpu.make_async_copy(src, dst, in_sem.at[len(copies)]))
    return copies[-1]

  def x_copy(i):
    rows = pl.ds(sum(X_CHUNKS[:i]), X_CHUNKS[i])
    return in_copy(x_hbm.at[rows], x_ref.at[rows])

  def start_copies(n):
    for _ in range(n):
      unstarted.pop(0).start()

  x0_cp = x_copy(0)
  wk_cp = [in_copy(wqkv_hbm.at[:, pl.ds(D + i * hd, hd)], wk_ref.at[:, pl.ds(i * hd, hd)]) for i in range(2)]
  x1_cp, x2_cp = x_copy(1), x_copy(2)
  wq_cp = in_copy(wqkv_hbm.at[:, pl.ds(0, D)], wq_ref)
  wv_cp = in_copy(wqkv_hbm.at[:, pl.ds(2 * D, D)], wv_ref)
  x3_cp = x_copy(3)
  late_cp = [in_copy(wo_hbm, wo_ref), in_copy(w1_hbm, w1_ref), in_copy(w2_hbm, w2_ref), in_copy(b1_hbm, b1_ref)]
  unstarted = list(copies)
  start_copies(4)
  one_ref[...] = jnp.ones(one_ref.shape, F32)

  def norm(r0):
    x = x_ref[r0:r0 + RB, :].astype(F32)
    xc = x - jnp.mean(x, axis=-1, keepdims=True)
    xn = xc * lax.rsqrt(jnp.mean(xc * xc, axis=-1, keepdims=True) + 1e-5)
    xn_ref[r0:r0 + RB, :] = xn.astype(BF16)
    top, bot = xn[:RB // 2], xn[RB // 2:]
    for i, op in enumerate(_strassen_lhs(top[:, :hd], top[:, hd:], bot[:, :hd], bot[:, hd:])):
      xs_ref[i, r0 // 2:(r0 + RB) // 2, :] = op.astype(BF16)

  def weight_jobs(w_ref, dst_ref):
    r, c = dst_ref.shape[1:]
    for t in range(0, r, JOB_ROWS):
      for u in range(0, c, 2 * LANES):
        def job(t=t, u=u, n=min(2 * LANES, c - u)):
          ops = _strassen_rhs(*[w_ref[i * r + t:i * r + t + JOB_ROWS, j * c + u:j * c + u + n].astype(F32)
                                for i in range(2) for j in range(2)])
          for i, op in enumerate(ops):
            dst_ref[i, t:t + JOB_ROWS, u:u + n] = op.astype(BF16)
          dep = (ops[0] + ops[6])[:, :LANES]
          return jnp.sum(dep.reshape(JOB_ROWS // 8, 8, LANES), axis=0)
        yield job

  jobs, jobs_per_dot = [], 0

  def with_jobs(x):
    n = min(jobs_per_dot, len(jobs))
    if not n:
      return _unpack(x)
    true = one_ref[:, :LANES] > 0
    parts = [x[t:t + 8, :LANES] for t in range(0, x.shape[0], 8)]
    for i in range(n):
      t = i * len(parts) // n
      parts[t] = _after(true, parts[t], jobs.pop(0)())
    return _unpack(jnp.concatenate([jnp.concatenate(parts, axis=0), x[:, LANES:]], axis=1))

  def project_k(r0):
    xn = xn_ref[r0:r0 + RB, :]
    return _dot(with_jobs(_pack(xn)) if jobs else xn, wk_ref[...]).astype(BF16)

  def store_k(r0, k):
    for h in range(HEADS):
      c, off = divmod(h * Dh, LANES)
      kt = _pack(k[:, c * LANES:(c + 1) * LANES])
      if off:
        kt = pltpu.roll(kt, LANES - off, 1)
      for t in range(RB // TK):
        j, tile = r0 // TK + t, kt[t * TK // 2:(t + 1) * TK // 2]
        k_ref[h, j] = tile[:8 * NM]
        kv_ref[h, j] = _unpack(tile[8 * NM:]).astype(F32)
        if j in EXTRA_TILES:
          kx_ref[h, EXTRA_TILES.index(j)] = _unpack(tile[8 * (NM - 1):8 * NM]).astype(F32)

  def project_q(qb):
    qT = _dot_nt(with_jobs(wqT_ref[...]), xn_ref[qb * TQ:(qb + 1) * TQ, :]) * q_scale
    qT_ref[qb] = qT.reshape(HEADS, Dh, TQ)

  def project_v(qb):
    xn = jnp.concatenate([xn_ref[t + o:t + o + 8, :]
                          for t in range(qb * TQ, (qb + 1) * TQ, TK) for o in P_ROWS], axis=0)
    vT = _dot_nt(with_jobs(wvT_ref[...]), xn)
    for t in range(TQ // TK):
      vT_ref[:, qb * (TQ // TK) + t] = vT[:, t * TK:(t + 1) * TK].reshape(HEADS, Dh, TK)

  def transpose(w_ref, dst_ref):
    for c in range(0, D, LANES):
      dst_ref[:, c:c + LANES] = _pack(w_ref[c:c + LANES, :].astype(F32).T.astype(BF16))

  x0_cp.wait()
  start_copies(1)
  norm(0)
  wk_cp[0].wait()
  k_left = _dot(xn_ref[0:RB, :], wk_ref[:, :hd]).astype(BF16)
  wk_cp[1].wait()
  x1_cp.wait()
  start_copies(1)
  ks = {0: jnp.concatenate([k_left, _dot(xn_ref[0:RB, :], wk_ref[:, hd:]).astype(BF16)], axis=1)}
  norm(RB)
  x2_cp.wait()
  start_copies(2)
  store_k(0, ks.pop(0))
  ks[1] = project_k(RB)
  norm(2 * RB)
  ks[2] = project_k(2 * RB)
  norm(3 * RB)
  wq_cp.wait()
  start_copies(2)
  transpose(wq_ref, wqT_ref)
  ks[3] = project_k(3 * RB)
  store_k(RB, ks.pop(1))
  project_q(0)
  wv_cp.wait()
  x3_cp.wait()
  start_copies(2)
  for op in PROJ_ORDER.split():
    kind, n = op[0], int(op[1:] or 0)
    if kind == "T":
      transpose(wv_ref, wvT_ref)
    elif kind == "n":
      norm(n * RB)
    elif kind == "k":
      ks[n] = project_k(n * RB)
    elif kind == "s":
      store_k(n * RB, ks.pop(n))
    elif kind == "q":
      project_q(n)
    elif kind == "v":
      project_v(n)
    else:
      for cp in late_cp:
        cp.wait()
      for w_ref, dst_ref in ((wo_ref, wos_ref), (w1_ref, w1s_ref), (w2_ref, w2s_ref)):
        jobs.extend(weight_jobs(w_ref, dst_ref))
      jobs_per_dot = -(-len(jobs) // n)
  assert not (jobs or ks or unstarted)

  steps = NK * NQ
  bad_ref[...] = jnp.zeros(bad_ref.shape, F32)
  p_ref[...] = jnp.zeros(p_ref.shape, F32)
  l_ref[...] = jnp.ones(l_ref.shape, F32)
  acc_ref[...] = jnp.zeros(acc_ref.shape, F32)

  def stage_keys(k16, slot, dims):
    for d in dims:
      kb_ref[slot, d] = jnp.broadcast_to(k16[:, d:d + 1], (16, LANES))

  def stage_queries(tab_ref, q8, col, d0, rows):
    for d in rows:
      tab_ref[col, d0 + d] = jnp.broadcast_to(q8[d:d + 1], (8, LANES))

  def vpu_scores(slot, tab_ref, col, hold):
    q = tab_ref[col]
    q = jnp.concatenate([hold(q[0])[None], q[1:]], axis=0)
    terms = kb_ref[slot].reshape(Dh, 2, 8, LANES) * q[:, None]
    return jnp.sum(terms, axis=0).reshape(16, LANES)

  def add_pv(u, h, r, p):
    j, qb = divmod(r, NQ)
    a = _dot(vT_ref[h, j], p)
    acc_ref[u, qb] = acc_ref[u, qb] + a if j > 0 else a

  def finish(u, h, qb, l):
    a = acc_ref[u, qb]
    l = jnp.broadcast_to(jnp.sum(l, axis=0, keepdims=True), (8, TQ))
    ok = (l >= 2.0 ** -60) & (l <= 2.0 ** 60) & (jnp.abs(a[:8]) + jnp.abs(a[8:]) <= 2.0 ** 120)
    bad = jnp.where(ok, bad_ref[...], 1.0)
    bad_ref[...] = bad
    inv = 1.0 / l
    lo, hi = a[:8] * inv, a[8:] * inv
    oT_ref[qb, h] = jnp.concatenate([lo, hi], axis=0)
    return lo + hi + bad

  stage_keys(kv_ref[0, 0], 0, range(Dh))
  stage_keys(kx_ref[0, 0], 2, range(Dh))
  for col in range(NQ * NC):
    for d0 in range(0, Dh, 8):
      q8 = qT_ref[col // NC, 0, d0:d0 + 8, (col % NC) * LANES:(col % NC + 1) * LANES]
      stage_queries(qa_ref, q8, col, d0, range(8))

  def head_pair(i, carry):
    true = one_ref[...] > 0
    true_tile = true[:, :LANES]
    scores, finished, extras = {}, {}, {}

    def from_slot(slot, c=0):
      if slot < 0:
        return lambda x: x
      s = scores[slot // NG]
      t = min(slot % NG, s.shape[0] // 16 - 1)
      return lambda x: _after(true_tile, x, s[16 * t:16 * t + 8, c * LANES:(c + 1) * LANES])

    def hold_keys(k16, g):
      return jnp.concatenate([from_slot(NG * g - KEY_LEAD)(k16[e:e + 8]) for e in (0, 8)], axis=0)

    heads = [jnp.maximum(2 * i - 1, 0), 2 * i, 2 * i + 1, jnp.minimum(2 * i + 2, HEADS - 1)]
    zero = lax.div(i, HEADS)
    pending = [(1, heads[0], steps - 1, p_ref[...])]
    for g in range(2 * steps):
      u, r = divmod(g, steps)
      j, qb = divmod(r, NQ)
      h_prev, h, h_next = heads[u:u + 3]
      tab_ref, tab_next = (qa_ref, qb_ref) if u == 0 else (qb_ref, qa_ref)

      q = qT_ref[qb, h]
      q_lo, q_hi = q[:8], q[8:]
      if g - FINISH_DUE in finished:
        q_lo = _after(true, q_lo, finished[g - FINISH_DUE])
      if g - EXTRA_DUE in extras:
        dep = jnp.concatenate(extras[g - EXTRA_DUE], axis=1)
        n = dep.shape[1]
        q_hi = jnp.concatenate([_after(true, q_hi[:, :n], dep)] + ([q_hi[:, n:]] if n < TQ else []), axis=1)
      q = jnp.concatenate([q_lo, q_hi], axis=0)

      n_mxu = NM - 1 if j in EXTRA_TILES else NM
      mxu_scores = lambda a, b: _dot(_unpack(k_ref[h, j, 8 * a:8 * b])[:, :Dh], q)
      if g > 0:
        s = mxu_scores(0, NG - n_mxu)
        add_pv(*pending.pop(0))
        s = jnp.concatenate([s, mxu_scores(NG - n_mxu, n_mxu)], axis=0)
      else:
        s = mxu_scores(0, n_mxu)
      scores[g] = s

      sv = jnp.concatenate(
          [vpu_scores(j % 2, tab_ref, qb * NC + c, from_slot(NG * g + CHAIN_SLOT[c], c))
           for c in range(NC)], axis=1)
      seg = sum(j > t for t in EXTRA_TILES)
      j0 = EXTRA_TILES[seg - 1] + 1 if seg else 0
      pos, span = r - j0 * NQ, (EXTRA_TILES[seg] - j0) * NQ
      par = (u * len(EXTRA_TILES) + seg) % 2
      for col in range(NQ * NC):
        if col * span // (NQ * NC) == pos:
          hold = from_slot(NG * g + EXTRA_SLOT - 2 * len(extras.get(g, [])))
          sx = vpu_scores(2 + par, tab_ref, col, hold)
          sx_ref[col // NC, :, (col % NC) * LANES:(col % NC + 1) * LANES] = sx
          extras.setdefault(g, []).extend([sx[:8], sx[8:]])

      if qb == NQ - 1 and pos // NQ < 4:
        k16 = kx_ref[h, seg + 1] if seg + 1 < len(EXTRA_TILES) else kx_ref[h_next, 0]
        d0 = 4 * (pos // NQ)
        stage_keys(hold_keys(k16, g), 3 - par, range(d0, d0 + 4))
      if KEY_STAGE[qb] < KEY_STAGE[qb + 1]:
        k16 = kv_ref[h, j + 1] if j + 1 < NK else kv_ref[h_next, 0]
        stage_keys(hold_keys(k16, g), (j + 1) % 2, range(KEY_STAGE[qb], KEY_STAGE[qb + 1]))
      d0 = 8 * (qb // 2)
      q8 = qT_ref[j // NC, h_next, d0:d0 + 8, (j % NC) * LANES:(j % NC + 1) * LANES]
      stage_queries(tab_next, from_slot(NG * g - QUERY_LEAD, 1)(q8), j + zero, d0,
                    range(4 * (qb % 2), 4 * (qb % 2) + 4))

      if g == 2 * steps - 1:
        add_pv(*pending.pop(0))
      if r in FINISH_STEPS:
        fq = FINISH_STEPS.index(r)
        l = jnp.concatenate([from_slot(NG * g - NG, c)(l_ref[1 - u, fq, :, c * LANES:(c + 1) * LANES])
                             for c in range(NC)], axis=1)
        finished[g] = finish(1 - u, h_prev, fq, l)

      rows = [s[:16 * VPU_POS], sv, s[16 * VPU_POS:]] + ([sx_ref[qb]] if n_mxu < NM else [])
      p = jnp.exp2(jnp.concatenate(rows, axis=0))
      sums = ([l_ref[u, qb][None]] if j > 0 else []) + [p.reshape(TK // 8, 8, TQ)]
      l_ref[u, qb] = jnp.sum(jnp.concatenate(sums, axis=0), axis=0)
      pending.append((u, h, r, jnp.concatenate([p[t:t + 8] for t in range(TK - 8, -1, -8)], axis=0)))
    p_ref[...] = pending.pop()[3]
    return carry

  lax.fori_loop(0, HEADS // 2, head_pair, 0)
  add_pv(1, HEADS - 1, steps - 1, p_ref[...])
  for qb in range(NQ):
    finish(1, HEADS - 1, qb, l_ref[1, qb])

  @pl.when(jnp.max(bad_ref[...]) > 0)
  def _():
    def redo(it, carry):
      h, qb = it // NQ, it % NQ
      q = qT_ref[qb, h]

      def score_tile(j, m):
        k = jnp.concatenate([k_ref[h, j], _pack(kv_ref[h, j].astype(BF16))], axis=0)
        s = _dot(_unpack(k)[:, :Dh], q)
        s = jnp.concatenate([s[o:o + 8] for o in P_ROWS], axis=0)
        s_ref[j] = s
        return jnp.maximum(m, jnp.max(s.reshape(TK // 8, 8, TQ), axis=0))

      m = lax.fori_loop(0, NK, score_tile, jnp.full((8, TQ), -jnp.inf, F32), unroll=True)
      m = jnp.max(m, axis=0, keepdims=True)

      def pv_tile(j, sums):
        p = jnp.exp2(s_ref[j] - m)
        return sums[0] + jnp.sum(p.reshape(TK // 8, 8, TQ), axis=0), sums[1] + _dot(vT_ref[h, j], p)

      l, a = lax.fori_loop(0, NK, pv_tile, (jnp.zeros((8, TQ), F32), jnp.zeros((Dh, TQ), F32)),
                           unroll=True)
      oT_ref[qb, h] = a / jnp.sum(l, axis=0, keepdims=True)
      return carry

    lax.fori_loop(0, HEADS * NQ, redo, 0)

  b1 = b1_ref[...].astype(F32).reshape(1, -1)

  def out_copy(i):
    rows = pl.ds(i * RB, RB)
    return pltpu.make_async_copy(out_ref.at[rows], out_hbm.at[rows], out_sem.at[i])

  def out_block(r, carry):
    m = TQ // 2
    xs = [xs_ref[i, pl.ds(pl.multiple_of(r * m, m), m), :] for i in range(7)]

    def hidden(c0, between):
      def prod(i):
        y = _dot(xs[i], w1s_ref[i, :, c0:c0 + LANES])
        between(i)
        return y
      act = [_mish(h + b1[:, (n % 2) * hf + c0:(n % 2) * hf + c0 + LANES])
             for n, h in enumerate(_strassen_blocks(prod))]
      ops = [op.astype(BF16) for op in _strassen_lhs(*act)]
      return lambda i, rows=slice(None): _dot(ops[i][rows], w2s_ref[i, c0:c0 + LANES, :])

    share = hidden(0, lambda i: None)
    o = oT_ref[r].reshape(D, TQ).T
    top, bot = [jnp.concatenate([o[t + e * RB // 2:t + (e + 1) * RB // 2] for t in range(0, TQ, RB)], axis=0)
                for e in range(2)]
    ops = _strassen_lhs(top[:, :hd], top[:, hd:], bot[:, :hd], bot[:, hd:])
    for i in STRASSEN_ORDER:
      m_ref[i] = _dot(ops[i].astype(BF16), wos_ref[i])
    for c0 in range(LANES, hf, LANES):
      def add_share(i, share=share):
        m_ref[i] += share(i)
      share = hidden(c0, add_share)
    for t in range(TQ // RB):
      sub = slice(t * RB // 2, (t + 1) * RB // 2)
      y = _strassen_blocks(lambda i: m_ref[i, sub] + share(i, sub))
      for e in range(2):
        rows = pl.ds(pl.multiple_of(r * TQ + t * RB + e * (RB // 2), RB // 2), RB // 2)
        res = x_ref[rows, :].astype(F32) + jnp.concatenate(y[2 * e:2 * e + 2], axis=1)
        out_ref[rows, :] = res.astype(out_ref.dtype)
      out_copy(r * (TQ // RB) + t).start()
    return carry

  lax.fori_loop(0, NQ, out_block, 0)
  for i in range(S // RB):
    out_copy(i).wait()


@jax.jit
def pallas_parallel_sum__mha_block__dense_activation_mish__prompt_kernel(
    A_x: jax.Array,
    A_wqkv: jax.Array,
    A_wo: jax.Array,
    B_x: jax.Array,
    B_w1: jax.Array,
    B_b1: jax.Array,
    B_w2: jax.Array,
):
  del B_x
  B, S, D = A_x.shape
  F = B_w1.shape[1]
  assert (B, S, D) == (1, sum(X_CHUNKS), 16 * HEADS) and F % (2 * LANES) == 0
  Dh, NQ, NK = D // HEADS, S // TQ, S // TK
  vmem = pltpu.VMEM
  hbm = pl.BlockSpec(memory_space=pl.ANY)
  out = pl.pallas_call(
      _kernel,
      out_shape=jax.ShapeDtypeStruct((S, D), A_x.dtype),
      in_specs=[hbm] * 6,
      out_specs=hbm,
      scratch_shapes=[
          vmem((S, D), A_x.dtype),
          *[vmem((D, D), A_wqkv.dtype)] * 3, vmem((D, D), A_wo.dtype),
          vmem((D, F), B_w1.dtype), vmem((F, D), B_w2.dtype), vmem((S, D), A_x.dtype),
          *[vmem((D // 2, D), U32)] * 2,
          vmem((S, D), BF16), vmem((7, S // 2, D // 2), BF16),
          vmem((7, D // 2, F // 2), BF16), vmem((7, F // 2, D // 2), BF16), vmem((7, D // 2, D // 2), BF16),
          vmem((NQ, HEADS, Dh, TQ), F32),
          vmem((HEADS, NK, 8 * NM, LANES), U32),
          vmem((HEADS, NK, 16, LANES), F32), vmem((HEADS, 4, 16, LANES), F32),
          vmem((HEADS, NK, Dh, TK), F32), vmem((NQ, HEADS, Dh, TQ), F32),
          *[vmem((S // LANES, Dh, 8, LANES), F32)] * 2, vmem((4, Dh, 16, LANES), F32),
          vmem((NQ, 16, TQ), F32), vmem((TK, TQ), F32),
          vmem((2, NQ, 8, TQ), F32), vmem((2, NQ, Dh, TQ), F32),
          vmem((8, TQ), F32), vmem((8, TQ), F32),
          vmem((NK, TK, TQ), F32), vmem((7, TQ // 2, D // 2), F32),
          vmem((F,), B_b1.dtype),
          pltpu.SemaphoreType.DMA((12,)), pltpu.SemaphoreType.DMA((S // RB,)),
      ],
      compiler_params=pltpu.CompilerParams(vmem_limit_bytes=100 * 2**20),
  )(A_x.reshape(S, D), A_wqkv, A_wo, B_w1, B_b1, B_w2)
  return out.reshape(B, S, D)
```
